```python
import os as _os
_os.environ.setdefault("JAX_PLATFORMS", "cpu")
import jax
import jax.numpy as jnp

def _softmax(x, axis=-1):
    return jax.nn.softmax(x, axis=axis)
def _gelu(x):
    return jax.nn.gelu(x, approximate=True)
def _silu(x):
    return jax.nn.silu(x)
def _sigmoid(x):
    return jax.nn.sigmoid(x)
def _layernorm(x, axis=-1, eps=1e-5):
    m = jnp.mean(x, axis=axis, keepdims=True)
    v = jnp.var(x, axis=axis, keepdims=True)
    return (x - m) / jnp.sqrt(v + eps)
def _scatter_add(tgt, idx, src, axis=0):
    return tgt.at[idx].add(src)
def _segment_sum(src, seg, n):
    return jax.ops.segment_sum(src, seg, n)
class _Rng:
    def __init__(self, key):
        self._k = key
    def _next(self):
        self._k, sub = jax.random.split(self._k)
        return sub
    def normal(self, shape):
        return jax.random.normal(self._next(), shape, dtype=jnp.bfloat16)
    def randint(self, lo, hi, shape):
        return jax.random.randint(self._next(), shape, lo, hi, dtype=jnp.int32)
    def uniform(self, shape, lo=0.0, hi=1.0):
        return jax.random.uniform(self._next(), shape, jnp.bfloat16, lo, hi)
    def permutation(self, n):
        return jax.random.permutation(self._next(), n)


kernel_name = 'sequential_preLN__ssm_conv_h3__dense_activation_gelu__prompt'

def setup_inputs():
    _rng = _Rng(jax.random.key(int.from_bytes(__import__("os").urandom(4), "little")))
    _w = (lambda a: (lambda t: t.astype(jnp.bfloat16) if jnp.issubdtype(t.dtype, jnp.floating) else t)(jnp.asarray(a)))
    def _A_setup():
        B, S, D = 1, 2048, 512
        ks = 4
        return {
            "q": _w((lambda *s: _rng.normal(s) * 0.05)(B, S, D)),
            "k": _w((lambda *s: _rng.normal(s) * 0.2)(B, S, D)),
            "v": _w((lambda *s: _rng.normal(s) * 0.2)(B, S, D)),
            "shift_k": _w((lambda *s: _rng.normal(s) * 0.2)(D, ks) * 0.5),
            "ssm_k": _w((lambda *s: _rng.normal(s) * 0.2)(D, S) * (1.0 / S ** 0.5)),
            "ssm_D": _w((lambda *s: _rng.normal(s) * 0.2)(D)),
        }
    _A_in = _A_setup()

    def _B_setup():
        B, S, D, F = 1, 2048, 512, 1376
        return {
            "x": _w((lambda *s: _rng.normal(s) * 0.05)(B, S, D)),
            "w1": _w((lambda *s: _rng.normal(s) * 0.2)(D, F) * (D ** -0.5)),
            "b1": _w((lambda *s: _rng.normal(s) * 0.2)(F) * 0.01),
            "w2": _w((lambda *s: _rng.normal(s) * 0.2)(F, D) * (F ** -0.5)),
            "b2": _w((lambda *s: _rng.normal(s) * 0.05)(D) * 0.01),
        }
    _B_in = _B_setup()

    return {
        "A_q": _A_in["q"],
        "A_k": _A_in["k"],
        "A_v": _A_in["v"],
        "A_shift_k": _A_in["shift_k"],
        "A_ssm_k": _A_in["ssm_k"],
        "A_ssm_D": _A_in["ssm_D"],
        "B_x": _B_in["x"],
        "B_w1": _B_in["w1"],
        "B_b1": _B_in["b1"],
        "B_w2": _B_in["w2"],
        "B_b2": _B_in["b2"],
    }

def reference(A_q, A_k, A_v, A_shift_k, A_ssm_k, A_ssm_D, B_x, B_w1, B_b1, B_w2, B_b2):
    def _A_ref(q, k, v, shift_k, ssm_k, ssm_D):
        B, S, D = q.shape
        ks = shift_k.shape[-1]
        k_pad = jnp.pad(k, ((0, 0), (ks - 1, 0), (0, 0)))
        k_shift = jnp.zeros_like(k)
        for t in range(ks):
            k_shift = k_shift + k_pad[:, t:t + S, :] * shift_k[:, ks - 1 - t][None, None, :]
        kv = k_shift * v
        L = 2 * S
        kv_pad = jnp.pad(kv, ((0, 0), (0, S), (0, 0)))
        kf_pad = jnp.pad(ssm_k, ((0, 0), (0, S)))
        kv_f = (lambda x, axes=(-2,-1): jnp.fft.rfft2(x.astype(jnp.float32), axes=axes))(kv_pad[:, None, :, :], axes=(1, 2))
        kf_f = (lambda x, axes=(-2,-1): jnp.fft.rfft2(x.astype(jnp.float32), axes=axes))(kf_pad[:, None, :], axes=(1, 2))
        kf_f = (lambda x, *d: x.transpose(*d))(kf_f, 1, 2, 0)
        y_f = kv_f * kf_f[None, :, :, :]
        y = (lambda x, s, axes=(-2,-1): jnp.fft.irfft2(x, s=s, axes=axes).astype(jnp.bfloat16))(y_f, (1, L), axes=(1, 2))[:, 0, :S, :]
        y = y + kv * ssm_D[None, None, :]
        return q * y

    def _B_ref(x, w1, b1, w2, b2):
        h = jnp.einsum("bsd,df->bsf", x, w1) + b1
        h = _gelu(h)
        return jnp.einsum("bsf,fd->bsd", h, w2) + b2

    x = A_q
    h = x + _A_ref(_layernorm(x, axis=-1), A_k, A_v, A_shift_k, A_ssm_k, A_ssm_D)
    h2 = h + _B_ref(_layernorm(h, axis=-1), B_w1, B_b1, B_w2, B_b2)
    return h2
```

```python
import contextlib
import functools
import os

import numpy as np
import jax
import jax.numpy as jnp
import jax.experimental.pallas as pl
import jax.experimental.pallas.tpu as pltpu

S, D, F = 2048, 512, 1376
KS = 4
B = 256
NB = S // B
N = 2 * B
NC = D // 128
NF = (F + 127) // 128
EPS = 1e-5
f32 = jnp.float32
bf16 = jnp.bfloat16
u32 = jnp.uint32


def _consts():
    th = 2.0 * np.pi / N
    k0 = np.concatenate([np.arange(0, 64, 2), np.arange(1, 64, 2)])

    def fmat(times):
        rows = []
        for h in range(2):
            ph = th * np.outer(k0 + 128 * h + 0.5, times)
            rows += [np.cos(ph), -np.sin(ph)]
        return np.concatenate(rows, 0)

    m = np.arange(64)
    l = np.arange(128)
    t_xe = 2 * l
    t_xo = 2 * l + 1
    t_ke = np.where(l % 2 == 0, l, 128 + (l - 1) % 128)
    t_ko = np.where(l % 2 == 1, l, 128 + (l - 1) % 128)
    gs = []
    for r in range(4):
        ph = th * np.outer(4 * m + r, k0 + 0.5)
        g = np.zeros((64, 128))
        g[:, 0::2] = np.cos(ph) * (2.0 / N)
        g[:, 1::2] = -np.sin(ph) * (2.0 / N)
        gs.append(g)
    mats = [fmat(t_ke), fmat(t_ko), fmat(t_xe), fmat(t_xo), np.concatenate(gs, 0)]
    return np.stack(mats, 0).astype(np.float32)


def _pack_rows_u32(a):
    u = np.ascontiguousarray(a, dtype=np.float32).view(np.uint32)
    b = (u + 0x7FFF + ((u >> 16) & 1)) >> 16
    return (b[..., 0::2, :] | (b[..., 1::2, :] << 16)).astype(np.uint32)


_CONSTS = _pack_rows_u32(_consts())


def _pk2(a, b):
    return pltpu.pack_elementwise([a, b], packed_dtype=bf16)


def _up(x):
    return pltpu.bitcast(x, bf16)


def _half(w, i):
    return pltpu.unpack_elementwise(w, index=i, packed_dtype=bf16, unpacked_dtype=f32)


ZX = NB
ZP = 0


def _ps(t):
    return t - 1


_FINAL = {
    0: [(0, 0)],
    1: [(1, 0), (0, 1), (ZX, 0), (ZX, 0)],
    2: [(2, 0), (0, 2), (1, 1), (ZX, 0)],
}
for _t in range(3, NB):
    _FINAL[_t] = [(_t, 0), (0, _t), (1, _t - 1), (_t - 1, 1)]
_FSRC = {0: [], 1: [ZP, ZP], 2: [ZP, ZP], 3: [ZP, ZP], 4: [_ps(2), ZP], 5: [_ps(3), ZP],
         6: [_ps(4), _ps(5)], 7: [_ps(6), _ps(7)]}
_EARLY = {
    1: ([(ZX, 0), (ZX, 0)], _ps(2)),
    2: ([(2, 2), (ZX, 0)], _ps(2)),
    3: ([(2, 3), (3, 2)], _ps(3)),
    4: ([(2, 4), (4, 2)], _ps(4)),
    5: ([(3, 3), (ZX, 0)], _ps(5)),
    6: ([(2, 5), (5, 2)], _ps(6)),
    7: ([(3, 4), (4, 3)], _ps(7)),
}
_LOOP = list(range(2, NB))

JS = 144
IO = 72
NR = 576
KOFF = 16
POFF = 8


def _rr(jp, k, n, off=0):
    return pl.ds(JS * jp + k + off, n)


def _ri(jp, k, n, off=0):
    return pl.ds(JS * jp + IO + k + off, n)


def _lut(t, table):
    if isinstance(t, int):
        return table[t]
    keys = sorted(table)
    out = jnp.int32(table[keys[-1]])
    for i in keys[-2::-1]:
        out = jnp.where(t == i, jnp.int32(table[i]), out)
    return out


def _ln(x):
    m = jnp.mean(x, axis=-1, keepdims=True)
    xc = x - m
    v = jnp.mean(xc * xc, axis=-1, keepdims=True)
    return xc * jax.lax.rsqrt(v + EPS)


_NT = (((1,), (1,)), ((), ()))
_GC0 = float(np.sqrt(2.0 / np.pi))
_GC1 = _GC0 * 0.044715
BODYONLY = int(os.environ.get("BODYONLY", 0))
SCOPES = int(os.environ.get("SCOPES", 0))
RC = 16
PU = 8


def _xor_all(vs):
    parts = []
    for v in vs:
        if v.dtype != u32:
            v = pltpu.bitcast(v, u32)
        for i in range(v.shape[0] // 8):
            for j in range(v.shape[1] // 128):
                parts.append(v[8 * i:8 * i + 8, 128 * j:128 * j + 128])
    while len(parts) > 1:
        parts = [parts[i] ^ parts[i + 1] if i + 1 < len(parts) else parts[i] for i in range(0, len(parts), 2)]
    return parts[0]


MX = os.environ.get(
    "MX", "b0 k0 x0 k1 k3 k2 Q0 x1 x2 Q2 b1 x3 Q1 b2 b3 Q3 b4 b5 b6 i0 b7 b8 b9 b10 m0 m1 m2 i1 i2 m3 m4 m5 i3 L0 m6 m7 L1").split()
MXL = "b0 b1 b2 b3 b4 b5 b6 b7 b8 b9 b10 m0 m1 m2 m3 m4 m5 m6 m7".split()
W1G = [0, 6, 11]
ILAG = int(os.environ.get("ILAG", -1))
PLAN = []


def _kernel(q_hbm, k_hbm, v_hbm, kk_hbm, sw_hbm, sd_hbm, c_hbm, w1_hbm, b1_hbm,
            w2_hbm, b2_hbm, o_hbm,
            kw, vw, qw, kkw, c_ref,
            xb, xf, ps, kp, kraw, ub, qn, hbs, hn, hs, gs, w1, w2, ob, kvd, sw_ref, sd_ref, b1_ref, b2_ref, zref,
            sem_in, sem_f, sem_o):

    def kk_copies(t0, t1, sem):
        return [pltpu.make_async_copy(kk_hbm.bitcast(u32).at[:, pl.ds(j * 128, 128)], kkw.at[j], sem)
                for j in range(2 * t0, 2 * t1)]

    def row_copies(src, dst, off, t0, t1, sem):
        n = (t1 - t0) * 128
        return [pltpu.make_async_copy(src.bitcast(u32).at[0, pl.ds(t0 * 128, n), pl.ds(128 * c, 128)],
                                      dst.at[c, pl.ds(off + t0 * 128, n), :], sem) for c in range(NC)]

    def kv_copies(t0, t1, sem):
        return row_copies(k_hbm, kw, 8, t0, t1, sem) + row_copies(v_hbm, vw, 0, t0, t1, sem)

    def q_copies(t0, t1, sem):
        return row_copies(q_hbm, qw, 0, t0, t1, sem)

    def w1_copies(g, sem):
        r0, r1 = 64 * W1G[g], min(64 * W1G[g + 1], F // 2)
        return [pltpu.make_async_copy(w1_hbm.bitcast(u32).at[pl.ds(r0, r1 - r0), pl.ds(128 * c, 128)],
                                      w1.at[c, pl.ds(r0, r1 - r0), :], sem) for c in range(NC)]

    def w2_copies(cp, sem):
        return [pltpu.make_async_copy(w2_hbm.bitcast(u32).at[:, pl.ds(128 * c, 128)], w2.at[c], sem)
                for c in (2 * cp, 2 * cp + 1)]

    def const_copy(lo, n, sem):
        return [pltpu.make_async_copy(c_hbm.at[pl.ds(lo, n)], c_ref.at[pl.ds(lo, n)], sem)]

    def small_copy(i, sem):
        s, d = [(sw_hbm, sw_ref), (sd_hbm, sd_ref), (b1_hbm, b1_ref), (b2_hbm, b2_ref)][i]
        return [pltpu.make_async_copy(s, d, sem)]

    def batch(i):
        sem = sem_in.at[i]
        if i == 0:
            return const_copy(0, 2, sem) + kk_copies(0, 1, sem) + q_copies(0, 1, sem)
        if i == 1:
            return small_copy(0, sem) + small_copy(1, sem) + kv_copies(0, 1, sem) + const_copy(2, 3, sem)
        if i == 2:
            return small_copy(2, sem) + small_copy(3, sem) + w1_copies(0, sem)
        if i == 3:
            return kk_copies(1, 2, sem) + kv_copies(1, 2, sem)
        if i == 4:
            return w1_copies(1, sem) + q_copies(1, 2, sem)
        if i in (5, 6):
            return w2_copies(i - 5, sem)
        t0, t1 = GRP[i - 7]
        return kk_copies(t0, t1, sem) + kv_copies(t0, t1, sem) + q_copies(t0, t1, sem)

    def fence():
        pl.semaphore_signal(sem_f, 1)
        pl.semaphore_wait(sem_f, 1)

    def out_copy(t, i=0, n=1):
        rows = pl.ds(t * B + i * (B // n), B // n)
        return pltpu.make_async_copy(ob.at[rows, :], o_hbm.at[0, rows, :], sem_o.at[0])

    def start(cps):
        for cp in cps:
            cp.start()

    cnt = [0]

    def wait(cps):
        cnt[0] += 1
        with (jax.named_scope("wait%d" % cnt[0]) if SCOPES else contextlib.nullcontext()):
            for cp in cps:
                cp.wait()

    def tie(x, toks):
        if not toks:
            return x
        mask = c_ref[4, pl.ds(0, 8), :] == jnp.uint32(0xFFFFFFFF)
        tok = _xor_all(toks)
        if x.dtype != u32:
            tok = pltpu.bitcast(tok, x.dtype)
        head_ = jnp.where(mask, tok, x[:8])
        return head_ if x.shape[0] == 8 else jnp.concatenate([head_, x[8:]], axis=0)

    def tie_at(x, row, toks):
        if not toks:
            return x
        if row == 0:
            return tie(x, toks)
        return jnp.concatenate([x[:row], tie(x[row:], toks)], axis=0)

    def a1_stage(t, z=None, withp=True):
        first = isinstance(t, int) and t == 0
        base = t * 128 if isinstance(t, int) else pl.multiple_of(t * 128, 128)
        sl = t % 2

        def planes(ref, c, off, m0, n):
            w0 = ref[c, pl.ds(off + base + 2 * m0, n, stride=2), :]
            w1_ = ref[c, pl.ds(off + base + 2 * m0 + 1, n, stride=2), :]
            return [_half(w0, 0), _half(w0, 1), _half(w1_, 0), _half(w1_, 1)]

        def ln1(rb, r, sp):
            rows = pl.ds(64 * r + RC * rb, RC)
            ws_ = [qw[c, pl.ds(base + 2 * RC * rb + r // 2, RC, stride=2), :] for c in range(NC)]
            ws_[0] = tie(ws_[0], sp)
            cols = [_half(w, r % 2) for w in ws_]
            y = _ln(jnp.concatenate(cols, axis=1))
            for c in range(NC):
                qn[c, rows, :] = y[:, 128 * c:128 * (c + 1)]
            if z is None:
                return None
            return [qn[z, pl.ds(64 * r + RC * rb, 8), :]]

        def conv(c, rb, sp):
            ls = slice(128 * c, 128 * (c + 1))
            ws = [sw_ref[j:j + 1, ls].astype(f32) for j in range(KS)]
            sd = sd_ref[pl.ds(128 * c, 128)].astype(f32)[None, :]
            m0 = PU * rb
            wm2 = kw[c, pl.ds(8 + base + 2 * m0 - 2, PU, stride=2), :]
            wm1 = tie(kw[c, pl.ds(8 + base + 2 * m0 - 1, PU, stride=2), :], sp)
            kd = [_half(wm2, 1), _half(wm1, 0), _half(wm1, 1)] + planes(kw, c, 8, m0, PU)
            vs = planes(vw, c, 0, m0, PU)
            kvs = []
            for r in range(4):
                ks = None
                for j in range(KS):
                    term = kd[3 + r - j] * ws[j]
                    ks = term if ks is None else ks + term
                kv = ks * vs[r]
                kvs.append(kv)
                kvd[c, pl.ds(64 * r + m0, PU), :] = kv * sd
            outs = []
            for p in range(2):
                pk = _pk2(kvs[p], kvs[p + 2])
                xb[c, p, pl.ds(m0, PU), :] = pk
            if z is None:
                return None
            return [xb[c + z, 0, pl.ds(m0, 8), :], kvd[c + z, pl.ds(m0, 8), :]]

        def xt(c, an):
            e0 = jnp.dot(_up(tie(c_ref[2], an[0])), _up(xb[c, 0]), preferred_element_type=f32)
            e1 = jnp.dot(_up(c_ref[3]), _up(xb[c, 1]), preferred_element_type=f32)
            for h in range(2):
                for part in range(2):
                    a = e0[128 * h + 64 * part:128 * h + 64 * part + 64]
                    b = e1[128 * h + 64 * part:128 * h + 64 * part + 64]
                    rw = _ri if part else _rr
                    xf[c][t, rw(h, 0, 64), :] = a + b
                    xf[c][t, rw(h + 2, 0, 64), :] = a - b

        def kt(c, an):
            rows = pl.ds(64 * c, 64)
            ka = kkw[2 * t, rows, :]
            kb = pltpu.roll(kkw[2 * t + 1, rows, :], 1, 1)
            ev = (jax.lax.broadcasted_iota(jnp.int32, ka.shape, 1) % 2) == 0
            ke = _up(jnp.where(ev, ka, kb))
            ko = _up(jnp.where(ev, kb, ka))
            e0 = jax.lax.dot_general(_up(tie(c_ref[0], an[0])), ke, _NT, preferred_element_type=f32)
            e1 = jax.lax.dot_general(_up(c_ref[1]), ko, _NT, preferred_element_type=f32)
            for half in range(2):
                kv_ = (e0 + e1) if half == 0 else (e0 - e1)
                for h in range(2):
                    jp = 2 * half + h
                    for par in range(2):
                        re = kv_[128 * h + 32 * par:128 * h + 32 * par + 32]
                        im = kv_[128 * h + 64 + 32 * par:128 * h + 64 + 32 * par + 32]
                        rs, is_ = _rr(jp, 32 * par, 32), _ri(jp, 32 * par, 32)
                        rk, ik = _rr(jp, 32 * par, 32, KOFF), _ri(jp, 32 * par, 32, KOFF)
                        if first:
                            kp[c][t, rk, :] = re
                            kp[c][t, ik, :] = im
                        else:
                            pr = kraw[c, rs, :]
                            pi = kraw[c, is_, :]
                            if par == 0:
                                kp[c][t, rk, :] = re - pi
                                kp[c][t, ik, :] = im + pr
                            else:
                                kp[c][t, rk, :] = re + pi
                                kp[c][t, ik, :] = im - pr
                        kraw[c, rs, :] = re
                        kraw[c, is_, :] = im

        units = {
            **{"P%d" % c: [functools.partial(conv, c, rb) for rb in range(64 // PU)] for c in range(NC)},
            **{"Q%d" % rb: [functools.partial(ln1, rb, r) for r in range(4)] for rb in range(64 // RC)},
        }
        mx = {}
        for i in range(4):
            mx["x%d" % i] = functools.partial(xt, i)
            mx["k%d" % i] = functools.partial(kt, i)
        need = {"x%d" % c: [("P%d" % c, 64 // PU - 1)] for c in range(NC)}
        return units, mx, need

    def a2_stage(t, z=None):
        sl = t % 2
        base = t * 128 if isinstance(t, int) else pl.multiple_of(t * 128, 128)
        if isinstance(t, int):
            fin = [p for p in _FINAL[t] if p[0] != ZX]
            fs = [s for s in _FSRC[t] if s != ZP]
            early = None
            if t in _EARLY and _EARLY[t][0][0][0] != ZX:
                early = [p for p in _EARLY[t][0] if p[0] != ZX]
                ed = _EARLY[t][1]
        else:
            fin = [(_lut(t, {s: _FINAL[s][u][0] for s in _LOOP}),
                    _lut(t, {s: _FINAL[s][u][1] for s in _LOOP})) for u in range(4)]
            fs = [_lut(t, {s: _FSRC[s][u] for s in _LOOP}) for u in range(2)]
            early = [(_lut(t, {s: _EARLY[s][0][u][0] for s in _LOOP}),
                      _lut(t, {s: _EARLY[s][0][u][1] for s in _LOOP})) for u in range(2)]
            ed = _lut(t, {s: _EARLY[s][1] for s in _LOOP})

        def cmac(zr, zi, pairs, c, jp, k, n, sp=None):
            for (i, j) in pairs:
                xr, xi = xf[c][i, _rr(jp, k, n), :], xf[c][i, _ri(jp, k, n), :]
                xr = tie(xr, sp)
                sp = None
                kr, ki = kp[c][j, _rr(jp, k, n, KOFF), :], kp[c][j, _ri(jp, k, n, KOFF), :]
                pr = xr * kr - xi * ki
                pi = xr * ki + xi * kr
                zr = pr if zr is None else zr + pr
                zi = pi if zi is None else zi + pi
            return zr, zi

        def earlyu(c, jp, sp):
            zr, zi = cmac(None, None, early, c, jp, 0, 64, sp)
            ps[c][ed, _rr(jp, 0, 64, POFF), :] = zr
            ps[c][ed, _ri(jp, 0, 64, POFF), :] = zi
            if z is None:
                return None
            return [ps[c][ed + z, _rr(jp, 0, 8, POFF), :]]

        def final(c, rb, sp):
            CF = 8
            zs = []
            for jp in range(4):
                zr = zi = None
                for s in fs:
                    a = ps[c][s, _rr(jp, CF * rb, CF, POFF), :]
                    b = ps[c][s, _ri(jp, CF * rb, CF, POFF), :]
                    zr = a if zr is None else zr + a
                    zi = b if zi is None else zi + b
                zs.append(cmac(zr, zi, fin, c, jp, CF * rb, CF, sp if jp == 0 else None))
            ar, ai = zs[0][0] + zs[2][0], zs[0][1] + zs[2][1]
            br, bi = zs[0][0] - zs[2][0], zs[0][1] - zs[2][1]
            cr, ci = zs[1][0] + zs[3][0], zs[1][1] + zs[3][1]
            dr, di = zs[1][0] - zs[3][0], zs[1][1] - zs[3][1]
            us = [(ar + cr, ai + ci), (br - di, bi + dr),
                  (ar - cr, ai - ci), (br + di, bi - dr)]
            outs = []
            for r in range(4):
                pk = _pk2(us[r][0], us[r][1])
                ub[c, r, pl.ds(CF * rb, CF), :] = pk
            if z is None:
                return None
            return [ub[c + z, 0, pl.ds(CF * rb, CF), :]]

        def idft(c, an):
            for r in range(4):
                y = jnp.dot(_up(c_ref[4, pl.ds(32 * r, 32), :]), _up(ub[c, r]), preferred_element_type=f32)
                rows = pl.ds(64 * r, 64)
                x = _half(qw[c, pl.ds(base + r // 2, 64, stride=2), :], r % 2)
                hs[sl, c, pl.ds(r, 64, stride=4), :] = x + qn[c, rows, :] * (y + kvd[c, rows, :])
            if z is None:
                return None
            return [hs[sl + z, c, pl.ds(0, 8), :]]

        def ln2(p, rb, sp):
            hns = []
            for r in (p, p + 2):
                nat = pl.ds(4 * RC * rb + r, RC, stride=4)
                cols = [hs[sl, c, nat, :] for c in range(NC)]
                cols[0] = tie(cols[0], sp)
                sp = None
                hns.append(_ln(jnp.concatenate(cols, axis=1)))
            pk = _pk2(hns[0], hns[1])
            for c in range(NC):
                hn[c, pl.ds(64 * p + RC * rb, RC), :] = pk[:, 128 * c:128 * (c + 1)]
            return None

        units = {
            **{"E%d" % c: [functools.partial(earlyu, c, jp) for jp in range(4)] if early else [] for c in range(NC)},
            **{"F%d" % c: [functools.partial(final, c, rb) for rb in range(8)] for c in range(NC)},
            **{"L%d" % p: [functools.partial(ln2, p, rb) for rb in range(64 // RC)] for p in range(2)},
        }
        mx = {"i%d" % i: functools.partial(idft, i) for i in range(4)}
        need = {"i%d" % c: [("E%d" % c, 3), ("F%d" % c, 7)] for c in range(NC)}
        return units, mx, need

    def b_stage(t):
        sl = t % 2
        obase = t * B if isinstance(t, int) else pl.multiple_of(t * B, B)

        def mm1(n, an):
            w = min(128, F - 128 * n)
            x0 = tie_at(tie(hn[0], an[0]), 64, an[1])
            x = _up(jnp.concatenate([x0] + [hn[c] for c in range(1, NC)], axis=1))
            wt = _up(jnp.concatenate([w1[c, pl.ds(64 * n, w // 2), :] for c in range(NC)], axis=1))
            h1 = jax.lax.dot_general(x, wt, _NT, preferred_element_type=f32)
            h1 = h1 + b1_ref[pl.ds(128 * n, w)].astype(f32)[None, :]
            u = h1 * (_GC0 + _GC1 * (h1 * h1))
            g = h1 + h1 * jnp.tanh(u)
            gs[n, :, pl.ds(0, w)] = _pk2(g[:128], g[128:])

        def mm2(i, an):
            cp, mq = i // 4, i % 4
            rp = pl.ds(32 * mq, 32)
            os_ = []
            for j in range(2):
                tiles = [gs[n, rp, :] for n in range(NF - 1)] + [gs[NF - 1, rp, pl.ds(0, F - 128 * (NF - 1))]]
                tiles[0] = tie(tiles[0], an[2 * j])
                tiles[6] = tie(tiles[6], an[2 * j + 1])
                g = _up(jnp.concatenate(tiles, axis=1))
                os_.append(jnp.dot(g, _up(w2[2 * cp + j]), preferred_element_type=f32))
            o = jnp.concatenate(os_, axis=1)
            rs = pl.ds(64 * mq, 64)
            hh = jnp.concatenate([hs[sl, 2 * cp, rs, :], hs[sl, 2 * cp + 1, rs, :]], axis=1)
            bb = b2_ref[pl.ds(256 * cp, 256)].astype(f32)[None, :]
            ob[pl.ds(obase + 64 * mq, 64), pl.ds(256 * cp, 256)] = ((0.5 * o + bb) + hh).astype(bf16)

        mx = {}
        for n in range(NF):
            mx["b%d" % n] = functools.partial(mm1, n)
        for i in range(8):
            mx["m%d" % i] = functools.partial(mm2, i)
        return {}, mx, {}

    AFTER = {}

    def run(order, plan, *stages):
        cnt[0] += 1
        with (jax.named_scope("run%d_%s" % (cnt[0], order[0])) if SCOPES else contextlib.nullcontext()):
            run_(order, plan, *stages)

    def run_(order, plan, *stages):
        units, mx, need = {}, {}, {}
        for u, m, n in stages:
            units.update(u)
            mx.update(m)
            need.update(n)
        exp = {"Q": ["Q0", "Q1", "Q2", "Q3"], "L": ["L0", "L1"]}
        order = [x for o in order for x in exp.get(o, [o])]
        assert all(o in mx or o in units for o in order), order
        plan = plan or []
        done, done_mx = set(), set()
        toks = {}
        state = {"sp": None, "j": 0}

        def emit(st, k, sp=None):
            if (st, k) in done or st not in units or k >= len(units[st]):
                return None
            for dep in AFTER.get(st, []):
                if isinstance(dep, tuple):
                    for kk in range(dep[1] + 1):
                        emit(dep[0], kk)
                else:
                    assert dep in done_mx or dep not in mx, (st, k, dep)
            for kk in range(k):
                emit(st, kk)
            outs = units[st][k]([sp] if sp is not None else None)
            done.add((st, k))
            return outs

        def link():
            j = state["j"]
            _, us, delay = plan[j]
            for (st, k, lag) in us:
                outs = emit(st, k, state["sp"])
                if outs is not None:
                    toks.setdefault(j + lag, []).extend(outs)
            parts = toks.get(j, [])
            if not parts and state["sp"] is not None:
                parts = [state["sp"]]
            if parts:
                v = _xor_all(parts)
                if delay < 0:
                    v = pltpu.roll(v, 1, 1)
                else:
                    v = pltpu.bitcast(v, f32)
                    for _ in range(delay):
                        v = jnp.tanh(v)
                state["sp"] = v
            state["j"] = j + 1

        for o in order:
            while state["j"] < len(plan) and plan[state["j"]][0] == o:
                link()
            if o in units:
                for k in range(len(units[o])):
                    emit(o, k)
                continue
            for dep in need.get(o, []):
                emit(*dep)
            outs = mx[o]([[]] * 5)
            done_mx.add(o)
            if outs is not None and plan and ILAG >= 0:
                toks.setdefault(state["j"] + ILAG, []).extend(outs)
        assert state["j"] == len(plan), plan[state["j"]]

    if BODYONLY:
        def body0(s, carry):
            z = zref[0]
            run(MX, PLAN, b_stage(s - 1), a2_stage(s, z), a1_stage(s, z))
            out_copy(s - 2).start()
            out_copy(s - 2).wait()
            return carry
        for i in range(10):
            start(batch(i))
            wait(batch(i))
        jax.lax.fori_loop(_LOOP[0], _LOOP[-1] + 1, body0, 0)
        return
    zref[0] = jnp.int32(0)
    for i in range(7):
        start(batch(i))
        fence()
    for c in range(NC):
        xf[c][ZX] = jnp.zeros(xf[c].shape[1:], f32)
        ps[c][ZP] = jnp.zeros(ps[c].shape[1:], f32)
        kw[c, pl.ds(0, 8), :] = jnp.zeros((8, 128), u32)
    wait(batch(0))
    run(PR[0], None, a1_stage(0))
    start(batch(7))
    wait(batch(1))
    run(PR[1], None, a1_stage(0), a2_stage(0))
    wait(batch(2))
    run(PR[2], None, b_stage(0))
    wait(batch(3))
    run(PR[3], None, a1_stage(1), b_stage(0))
    start(batch(8))
    wait(batch(4))
    run(PR[4], None, a1_stage(1), a2_stage(1), b_stage(0))
    start(batch(9))
    wait(batch(5))
    run(PR[5], None, a2_stage(1), b_stage(0))
    wait(batch(6))
    run(PR[6], None, b_stage(0))
    wait(batch(7))

    def body(s, carry):
        out_copy(s - 2).start()
        for gi in (1, 2):
            @pl.when(s == GRP[gi][0])
            def _():
                wait(batch(7 + gi))
        z = zref[0]
        run(MX, PLAN, b_stage(s - 1), a2_stage(s, z), a1_stage(s, z))
        return carry

    jax.lax.fori_loop(_LOOP[0], _LOOP[-1] + 1, body, 0)

    out_copy(NB - 2).start()
    run(MXL, None, b_stage(NB - 1))
    out_copy(NB - 1).start()
    wait([out_copy(t) for t in range(NB)])


PR = [x.split() for x in os.environ.get(
    "PR", "k0 k1 Q k2 k3|x0 x1 x2 x3 i0 i1 i2 i3 L|b0 b1 b2 b3|k0 k1 b4 x0 k2 x1 k3 x2 b5 x3|"
    "Q b6 b7 i0 b8 i1 b9 i2 b10 i3|L m0 m1 m2 m3|m4 m5 m6 m7").split("|")]
GRP = [(2, 3), (3, 5), (5, 8)]
FT = int(os.environ.get("FT", 1))


@jax.jit
def pallas_sequential_preLN__ssm_conv_h3__dense_activation_gelu__prompt_kernel(
    A_q, A_k, A_v, A_shift_k, A_ssm_k, A_ssm_D, B_x, B_w1, B_b1, B_w2, B_b2,
):
    del B_x
    consts = jnp.asarray(_CONSTS)
    any_spec = pl.BlockSpec(memory_space=pl.ANY)
    scratch = [
        pltpu.VMEM((NC, S // 2 + 8, 128), u32),
        pltpu.VMEM((NC, S // 2, 128), u32),
        pltpu.VMEM((NC, S // 2, 128), u32),
        pltpu.VMEM((S // 128, D // 2, 128), u32),
        pltpu.VMEM((5, 128, 128), u32),
        pltpu.VMEM((NC, 2, 64, 128), u32),
        [pltpu.VMEM((NB + 1, NR, 128), f32)] * NC,
        [pltpu.VMEM((7, NR + 32, 128), f32)] * NC,
        [pltpu.VMEM((NB, NR + 32, 128), f32)] * NC,
        pltpu.VMEM((NC, NR, 128), f32),
        pltpu.VMEM((NC, 4, 64, 128), u32),
        pltpu.VMEM((NC, B, 128), f32),
        pltpu.VMEM((NC, B, 128), f32),
        pltpu.VMEM((NC, B // 2, 128), u32),
        pltpu.VMEM((2, NC, B, 128), f32),
        pltpu.VMEM((NF, B // 2, 128), u32),
        pltpu.VMEM((NC, F // 2, 128), u32),
        pltpu.VMEM((NC, F // 2, 128), u32),
        pltpu.VMEM((S, D), bf16),
        pltpu.VMEM((NC, B, 128), f32),
        pltpu.VMEM((KS, D), bf16),
        pltpu.VMEM((D,), bf16),
        pltpu.VMEM((F,), bf16),
        pltpu.VMEM((D,), bf16),
        pltpu.SMEM((1,), jnp.int32),
        pltpu.SemaphoreType.DMA((10,)),
        pltpu.SemaphoreType.REGULAR,
        pltpu.SemaphoreType.DMA((1,)),
    ]
    return pl.pallas_call(
        _kernel,
        in_specs=[any_spec] * 11,
        out_specs=any_spec,
        out_shape=jax.ShapeDtypeStruct((1, S, D), bf16),
        scratch_shapes=scratch,
        compiler_params=pltpu.CompilerParams(
            vmem_limit_bytes=100 * 1024 * 1024,
            disable_bounds_checks=True,
        ),
    )(A_q, A_k, A_v, A_ssm_k, A_shift_k.T, A_ssm_D, consts, B_w1.T, B_b1, B_w2, B_b2)
```

```python
import functools

import numpy as np
import jax
import jax.numpy as jnp
import jax.experimental.pallas as pl
import jax.experimental.pallas.tpu as pltpu

S, D, F = 2048, 512, 1376
KS = 4
B = 256
NB = S // B
N = 2 * B
NC = D // 128
NF = (F + 127) // 128
EPS = 1e-5
f32 = jnp.float32
bf16 = jnp.bfloat16
u32 = jnp.uint32


def _pk2(a, b):
    return pltpu.pack_elementwise([a, b], packed_dtype=bf16)


def _up(x):
    return pltpu.bitcast(x, bf16)


def _half(w, i):
    return pltpu.unpack_elementwise(w, index=i, packed_dtype=bf16, unpacked_dtype=f32)


ZX = NB
ZP = 0


def _ps(t):
    return t - 1


_FINAL = {
    0: [(0, 0)],
    1: [(1, 0), (0, 1)],
    2: [(2, 0), (0, 2), (1, 1), (ZX, 0)],
}
for _t in range(3, NB):
    _FINAL[_t] = [(_t, 0), (0, _t), (1, _t - 1), (_t - 1, 1)]
_FSRC = {0: [], 1: [], 2: [ZP, ZP], 3: [ZP, ZP], 4: [_ps(2), ZP], 5: [_ps(3), ZP],
         6: [_ps(4), _ps(5)], 7: [_ps(6), _ps(7)]}
_EARLY = {
    2: ([(2, 2), (ZX, 0)], _ps(2)),
    3: ([(2, 3), (3, 2)], _ps(3)),
    4: ([(2, 4), (4, 2)], _ps(4)),
    5: ([(3, 3), (ZX, 0)], _ps(5)),
    6: ([(2, 5), (5, 2)], _ps(6)),
    7: ([(3, 4), (4, 3)], _ps(7)),
}
_LOOP = list(range(2, NB))

JS = 144
IO = 72
NR = 576
KOFF = 16
POFF = 8


def _rr(jp, k, n, off=0):
    return pl.ds(JS * jp + k + off, n)


def _ri(jp, k, n, off=0):
    return pl.ds(JS * jp + IO + k + off, n)


def _lut(t, table):
    keys = sorted(table)
    out = jnp.int32(table[keys[-1]])
    for i in keys[-2::-1]:
        out = jnp.where(t == i, jnp.int32(table[i]), out)
    return out


def _ln(x):
    m = jnp.mean(x, axis=-1, keepdims=True)
    xc = x - m
    v = jnp.mean(xc * xc, axis=-1, keepdims=True)
    return xc * jax.lax.rsqrt(v + EPS)


_SINC = [1.0, -1.0 / 6, 1.0 / 120, -1.0 / 5040, 1.0 / 362880, -1.0 / 39916800]
_NT = (((1,), (1,)), ((), ()))
_GC0 = float(np.sqrt(2.0 / np.pi))
_GC1 = _GC0 * 0.044715
RC = 16
PU = 8
PAD = 32

MX = ("b0 k0 x0 Q2 k3 k2 x1 k1 x3 b1 x2 Q1 Q0 b2 b3 b4 b5 Q3 i0 b6 b7 b8 b9 b10 "
      "m0 m1 i2 i3 m2 i1 m3 L0 m4 m5 L1 m6 m7").split()
PR = [x.split() for x in (
    "k0 k1 Q0 Q1 Q2 Q3 k3 k2|x0 x1 i0 x2 x3 i1 i2 i3 L0 L1|b0 b1 b2 b3|"
    "b4 k0 x0 k1 x1 k2 x2 k3 x3 b5|Q0 Q2 Q1 Q3 b6 i0 b7 b8 i1 b9 i2 b10 i3|"
    "m2 L1 L0 m0 m1 m3|m4 m5 m6 m7").split("|")]
W1G = [0, 6, 11]
GRP = [(2, 3), (3, 5), (5, 8)]


def _kernel(q_hbm, k_hbm, v_hbm, kk_hbm, sw_hbm, sd_hbm, w1_hbm, b1_hbm, w2_hbm, b2_hbm, o_hbm,
            kw, vw, qw, kkw, c_ref, xb, xf, ps, kp, kraw, ub, qn, hn, hs, gs, w1, w2, ob, kvd,
            sw_ref, sd_ref, b1_ref, b2_ref, sem_in, sem_f, sem_o):

    def kk_copies(t0, t1, sem):
        return [pltpu.make_async_copy(kk_hbm.bitcast(u32).at[:, pl.ds(j * 128, 128)], kkw.at[j], sem)
                for j in range(2 * t0, 2 * t1)]

    def row_copies(src, dst, off, t0, t1, sem):
        n = (t1 - t0) * 128
        return [pltpu.make_async_copy(src.bitcast(u32).at[0, pl.ds(t0 * 128, n), pl.ds(128 * c, 128)],
                                      dst.at[c, pl.ds(off + t0 * 128, n), :], sem) for c in range(NC)]

    def kv_copies(t0, t1, sem):
        return row_copies(k_hbm, kw, 8, t0, t1, sem) + row_copies(v_hbm, vw, 0, t0, t1, sem)

    def q_copies(t0, t1, sem):
        return row_copies(q_hbm, qw, 0, t0, t1, sem)

    def w1_copies(g, sem):
        r0, r1 = 64 * W1G[g], min(64 * W1G[g + 1], F // 2)
        return [pltpu.make_async_copy(w1_hbm.bitcast(u32).at[pl.ds(r0, r1 - r0), pl.ds(128 * c, 128)],
                                      w1.at[c, pl.ds(r0, r1 - r0), :], sem) for c in range(NC)]

    def w2_copies(cp, sem):
        return [pltpu.make_async_copy(w2_hbm.bitcast(u32).at[:, pl.ds(128 * c, 128)], w2.at[c], sem)
                for c in (2 * cp, 2 * cp + 1)]

    def small_copy(i, sem):
        s, d = [(sw_hbm, sw_ref), (sd_hbm, sd_ref), (b1_hbm, b1_ref), (b2_hbm, b2_ref)][i]
        return [pltpu.make_async_copy(s, d, sem)]

    def batch(i):
        sem = sem_in.at[i]
        if i == 0:
            return kk_copies(0, 1, sem) + q_copies(0, 1, sem)
        if i == 1:
            return small_copy(0, sem) + small_copy(1, sem) + kv_copies(0, 1, sem)
        if i == 2:
            return small_copy(2, sem) + small_copy(3, sem) + w1_copies(0, sem)
        if i == 3:
            return kk_copies(1, 2, sem) + kv_copies(1, 2, sem)
        if i == 4:
            return w1_copies(1, sem) + q_copies(1, 2, sem)
        if i in (5, 6):
            return w2_copies(i - 5, sem)
        t0, t1 = GRP[i - 7]
        return kk_copies(t0, t1, sem) + kv_copies(t0, t1, sem) + q_copies(t0, t1, sem)

    def fence():
        pl.semaphore_signal(sem_f, 1)
        pl.semaphore_wait(sem_f, 1)

    def out_copy(t, i=0, n=1):
        rows = pl.ds(t * B + i * (B // n), B // n)
        return pltpu.make_async_copy(ob.at[rows, :], o_hbm.at[0, rows, :], sem_o.at[0])

    def start(cps):
        for cp in cps:
            cp.start()

    def wait(cps):
        for cp in cps:
            cp.wait()

    def gen_consts():
        row = jax.lax.broadcasted_iota(jnp.int32, (32, 128), 0)
        lane = jax.lax.broadcasted_iota(jnp.int32, (32, 128), 1)

        def k0_of(i):
            return jnp.where(i < 32, 2 * i, 2 * i - 63)

        def cosp(p, scale=1.0):
            q = (((p + 512) & 1023) - 512).astype(f32)
            y = (256.0 - jnp.abs(q)) * (np.pi / 512)
            u = y * y
            acc = _SINC[-1] * scale
            for cf in _SINC[-2::-1]:
                acc = acc * u + cf * scale
            return acc * y

        wrap = 128 + ((lane + 127) & 127)
        times = [jnp.where(lane % 2 == 0, lane, wrap), jnp.where(lane % 2 == 1, lane, wrap),
                 2 * lane, 2 * lane + 1]
        for mi in range(4):
            tm = times[mi]
            sg = jnp.where((tm & 2) == 0, 1.0, -1.0)
            re, im = [], []
            for odd in range(2):
                p = (2 * k0_of(2 * row + odd) + 1) * tm
                re.append(cosp(p))
                im.append(cosp(p + 256))
            c_ref[mi, pl.ds(0, 32), :] = _pk2(re[0], re[1])
            c_ref[mi, pl.ds(32, 32), :] = _pk2(im[0], im[1])
            if mi % 2 == 0:
                c_ref[mi, pl.ds(64, 32), :] = _pk2(re[0] * sg, re[1] * sg)
                c_ref[mi, pl.ds(96, 32), :] = _pk2(im[0] * sg, im[1] * sg)
            else:
                c_ref[mi, pl.ds(64, 32), :] = _pk2(im[0] * sg, im[1] * sg)
                c_ref[mi, pl.ds(96, 32), :] = _pk2(re[0] * (-sg), re[1] * (-sg))
        f2 = 2 * k0_of(lane // 2) + 1
        ph = jnp.where(lane % 2 == 1, 256, 0)
        for r in range(4):
            halves = [cosp(f2 * (4 * (2 * row + odd) + r) + ph, 2.0 / N) for odd in range(2)]
            c_ref[4, pl.ds(32 * r, 32), :] = _pk2(halves[0], halves[1])

    def a1_stage(t):
        first = isinstance(t, int) and t == 0
        base = t * 128 if isinstance(t, int) else pl.multiple_of(t * 128, 128)

        def planes(ref, c, off, m0, n):
            w0 = ref[c, pl.ds(off + base + 2 * m0, n, stride=2), :]
            w1_ = ref[c, pl.ds(off + base + 2 * m0 + 1, n, stride=2), :]
            return [_half(w0, 0), _half(w0, 1), _half(w1_, 0), _half(w1_, 1)]

        def ln1(rb, r):
            rows = pl.ds(64 * r + RC * rb, RC)
            cols = [_half(qw[c, pl.ds(base + 2 * RC * rb + r // 2, RC, stride=2), :], r % 2)
                    for c in range(NC)]
            y = _ln(jnp.concatenate(cols, axis=1))
            for c in range(NC):
                qn[c, rows, :] = y[:, 128 * c:128 * (c + 1)]

        def conv(c, rb):
            ls = slice(128 * c, 128 * (c + 1))
            ws = [sw_ref[j:j + 1, ls].astype(f32) for j in range(KS)]
            sd = sd_ref[pl.ds(128 * c, 128)].astype(f32)[None, :]
            m0 = PU * rb
            wm2 = kw[c, pl.ds(8 + base + 2 * m0 - 2, PU, stride=2), :]
            wm1 = kw[c, pl.ds(8 + base + 2 * m0 - 1, PU, stride=2), :]
            kd = [_half(wm2, 1), _half(wm1, 0), _half(wm1, 1)] + planes(kw, c, 8, m0, PU)
            vs = planes(vw, c, 0, m0, PU)
            kvs = []
            for r in range(4):
                ks = None
                for j in range(KS):
                    term = kd[3 + r - j] * ws[j]
                    ks = term if ks is None else ks + term
                kv = ks * vs[r]
                kvs.append(kv)
                kvd[c, pl.ds(64 * r + m0, PU), :] = kv * sd
            for p in range(2):
                xb[c, p, pl.ds(m0, PU), :] = _pk2(kvs[p], kvs[p + 2])

        def xt(c):
            e0 = jnp.dot(_up(c_ref[2]), _up(xb[c, 0]), preferred_element_type=f32)
            e1 = jnp.dot(_up(c_ref[3]), _up(xb[c, 1]), preferred_element_type=f32)
            for h in range(2):
                for part in range(2):
                    a = e0[128 * h + 64 * part:128 * h + 64 * part + 64]
                    b = e1[128 * h + 64 * part:128 * h + 64 * part + 64]
                    rw = _ri if part else _rr
                    xf[c][t, rw(h, 0, 64), :] = a + b
                    xf[c][t, rw(h + 2, 0, 64), :] = a - b

        def kt(c):
            rows = pl.ds(64 * c, 64)
            ka = kkw[2 * t, rows, :]
            kb = pltpu.roll(kkw[2 * t + 1, rows, :], 1, 1)
            ev = (jax.lax.broadcasted_iota(jnp.int32, ka.shape, 1) % 2) == 0
            ke = _up(jnp.where(ev, ka, kb))
            ko = _up(jnp.where(ev, kb, ka))
            e0 = jax.lax.dot_general(_up(c_ref[0]), ke, _NT, preferred_element_type=f32)
            e1 = jax.lax.dot_general(_up(c_ref[1]), ko, _NT, preferred_element_type=f32)
            for half in range(2):
                kv_ = (e0 + e1) if half == 0 else (e0 - e1)
                for h in range(2):
                    jp = 2 * half + h
                    for par in range(2):
                        re = kv_[128 * h + 32 * par:128 * h + 32 * par + 32]
                        im = kv_[128 * h + 64 + 32 * par:128 * h + 64 + 32 * par + 32]
                        rs, is_ = _rr(jp, 32 * par, 32), _ri(jp, 32 * par, 32)
                        rk, ik = _rr(jp, 32 * par, 32, KOFF), _ri(jp, 32 * par, 32, KOFF)
                        if first:
                            kp[c][t, rk, :] = re
                            kp[c][t, ik, :] = im
                        else:
                            pr = kraw[c, rs, :]
                            pi = kraw[c, is_, :]
                            if par == 0:
                                kp[c][t, rk, :] = re - pi
                                kp[c][t, ik, :] = im + pr
                            else:
                                kp[c][t, rk, :] = re + pi
                                kp[c][t, ik, :] = im - pr
                        kraw[c, rs, :] = re
                        kraw[c, is_, :] = im

        units = {}
        mx = {}
        for c in range(NC):
            units["P%d" % c] = [functools.partial(conv, c, rb) for rb in range(64 // PU)]
            mx["x%d" % c] = functools.partial(xt, c)
            mx["k%d" % c] = functools.partial(kt, c)
        for rb in range(64 // RC):
            units["Q%d" % rb] = [functools.partial(ln1, rb, r) for r in range(4)]
        need = {"x%d" % c: ["P%d" % c] for c in range(NC)}
        return units, mx, need

    def a2_stage(t):
        sl = t % 2
        if isinstance(t, int):
            base = t * 128
            fin, fs, early = _FINAL[t], _FSRC[t], None
        else:
            base = pl.multiple_of(t * 128, 128)
            fin = [(_lut(t, {s: _FINAL[s][u][0] for s in _LOOP}),
                    _lut(t, {s: _FINAL[s][u][1] for s in _LOOP})) for u in range(4)]
            fs = [_lut(t, {s: _FSRC[s][u] for s in _LOOP}) for u in range(2)]
            early = [(_lut(t, {s: _EARLY[s][0][u][0] for s in _LOOP}),
                      _lut(t, {s: _EARLY[s][0][u][1] for s in _LOOP})) for u in range(2)]
            ed = _lut(t, {s: _EARLY[s][1] for s in _LOOP})

        def cmac(zr, zi, pairs, c, jp, k, n):
            for (i, j) in pairs:
                xr, xi = xf[c][i, _rr(jp, k, n), :], xf[c][i, _ri(jp, k, n), :]
                kr, ki = kp[c][j, _rr(jp, k, n, KOFF), :], kp[c][j, _ri(jp, k, n, KOFF), :]
                pr = xr * kr - xi * ki
                pi = xr * ki + xi * kr
                zr = pr if zr is None else zr + pr
                zi = pi if zi is None else zi + pi
            return zr, zi

        def earlyu(c, jp):
            zr, zi = cmac(None, None, early, c, jp, 0, 64)
            ps[c][ed, _rr(jp, 0, 64, POFF), :] = zr
            ps[c][ed, _ri(jp, 0, 64, POFF), :] = zi

        def final(c, rb):
            zs = []
            for jp in range(4):
                zr = zi = None
                for s in fs:
                    a = ps[c][s, _rr(jp, 8 * rb, 8, POFF), :]
                    b = ps[c][s, _ri(jp, 8 * rb, 8, POFF), :]
                    zr = a if zr is None else zr + a
                    zi = b if zi is None else zi + b
                zs.append(cmac(zr, zi, fin, c, jp, 8 * rb, 8))
            ar, ai = zs[0][0] + zs[2][0], zs[0][1] + zs[2][1]
            br, bi = zs[0][0] - zs[2][0], zs[0][1] - zs[2][1]
            cr, ci = zs[1][0] + zs[3][0], zs[1][1] + zs[3][1]
            dr, di = zs[1][0] - zs[3][0], zs[1][1] - zs[3][1]
            us = [(ar + cr, ai + ci), (br - di, bi + dr),
                  (ar - cr, ai - ci), (br + di, bi - dr)]
            for r in range(4):
                ub[c, r, pl.ds(8 * rb, 8), :] = _pk2(us[r][0], us[r][1])

        def idft(c):
            for r in range(4):
                y = jnp.dot(_up(c_ref[4, pl.ds(32 * r, 32), :]), _up(ub[c, r]), preferred_element_type=f32)
                rows = pl.ds(64 * r, 64)
                x = _half(qw[c, pl.ds(base + r // 2, 64, stride=2), :], r % 2)
                hs[sl, c, pl.ds(r, 64, stride=4), :] = x + qn[c, rows, :] * (y + kvd[c, rows, :])

        def ln2(p, rb):
            hns = []
            for r in (p, p + 2):
                nat = pl.ds(4 * RC * rb + r, RC, stride=4)
                hns.append(_ln(jnp.concatenate([hs[sl, c, nat, :] for c in range(NC)], axis=1)))
            pk = _pk2(hns[0], hns[1])
            for c in range(NC):
                hn[c, pl.ds(64 * p + RC * rb, RC), :] = pk[:, 128 * c:128 * (c + 1)]

        units = {}
        mx = {}
        for c in range(NC):
            units["E%d" % c] = [functools.partial(earlyu, c, jp) for jp in range(4)] if early else []
            units["F%d" % c] = [functools.partial(final, c, rb) for rb in range(8)]
            mx["i%d" % c] = functools.partial(idft, c)
        for p in range(2):
            units["L%d" % p] = [functools.partial(ln2, p, rb) for rb in range(64 // RC)]
        need = {"i%d" % c: ["E%d" % c, "F%d" % c] for c in range(NC)}
        return units, mx, need

    def b_stage(t):
        sl = t % 2
        obase = t * B if isinstance(t, int) else pl.multiple_of(t * B, B)

        def mm1(n):
            w = min(128, F - 128 * n)
            x = _up(jnp.concatenate([hn[c] for c in range(NC)], axis=1))
            wt = _up(jnp.concatenate([w1[c, pl.ds(64 * n, w // 2), :] for c in range(NC)], axis=1))
            h1 = jax.lax.dot_general(x, wt, _NT, preferred_element_type=f32)
            h1 = h1 + b1_ref[pl.ds(128 * n, w)].astype(f32)[None, :]
            u = h1 * (_GC0 + _GC1 * (h1 * h1))
            g = h1 + h1 * jnp.tanh(u)
            gs[n, :, pl.ds(0, w)] = _pk2(g[:128], g[128:])

        def mm2(i):
            cp, mq = i // 4, i % 4
            rp = pl.ds(32 * mq, 32)
            tiles = [gs[n, rp, :] for n in range(NF - 1)] + [gs[NF - 1, rp, pl.ds(0, F - 128 * (NF - 1))]]
            g = _up(jnp.concatenate(tiles, axis=1))
            o = jnp.concatenate([jnp.dot(g, _up(w2[2 * cp + j]), preferred_element_type=f32)
                                 for j in range(2)], axis=1)
            rs = pl.ds(64 * mq, 64)
            hh = jnp.concatenate([hs[sl, 2 * cp, rs, :], hs[sl, 2 * cp + 1, rs, :]], axis=1)
            bb = b2_ref[pl.ds(256 * cp, 256)].astype(f32)[None, :]
            ob[pl.ds(obase + 64 * mq, 64), pl.ds(256 * cp, 256)] = ((0.5 * o + bb) + hh).astype(bf16)

        mx = {}
        for n in range(NF):
            mx["b%d" % n] = functools.partial(mm1, n)
        for i in range(8):
            mx["m%d" % i] = functools.partial(mm2, i)
        return {}, mx, {}

    def run(order, *stages):
        units, mx, need = {}, {}, {}
        for u, m, n in stages:
            units.update(u)
            mx.update(m)
            need.update(n)
        for o in order:
            if o in units:
                for fn in units[o]:
                    fn()
            else:
                for st in need.get(o, []):
                    for fn in units[st]:
                        fn()
                mx[o]()

    for i in range(7):
        start(batch(i))
        fence()
    for c in range(NC):
        xf[c][ZX] = jnp.zeros(xf[c].shape[1:], f32)
        ps[c][ZP] = jnp.zeros(ps[c].shape[1:], f32)
        kw[c, pl.ds(0, 8), :] = jnp.zeros((8, 128), u32)
    gen_consts()
    wait(batch(0))
    run(PR[0], a1_stage(0))
    start(batch(7))
    wait(batch(1))
    run(PR[1], a1_stage(0), a2_stage(0))
    wait(batch(2))
    run(PR[2], b_stage(0))
    wait(batch(3))
    run(PR[3], a1_stage(1), b_stage(0))
    start(batch(8))
    wait(batch(4))
    run(PR[4], a1_stage(1), a2_stage(1), b_stage(0))
    start(batch(9))
    wait(batch(5))
    run(PR[5], a2_stage(1), b_stage(0))
    wait(batch(6))
    run(PR[6], b_stage(0))
    wait(batch(7))

    def body(it, carry):
        s = _LOOP[0] + it
        out_copy(s - 2).start()
        for gi in (1, 2):
            @pl.when(s == GRP[gi][0])
            def _():
                wait(batch(7 + gi))
        run(MX, b_stage(s - 1), a2_stage(s), a1_stage(s))
        return carry

    jax.lax.fori_loop(0, len(_LOOP), body, 0)

    out_copy(NB - 2).start()
    run(["b%d" % n for n in range(NF)], b_stage(NB - 1))
    for mq in range(4):
        run(["m%d" % mq, "m%d" % (mq + 4)], b_stage(NB - 1))
        out_copy(NB - 1, mq, 4).start()
    wait([out_copy(t) for t in range(NB - 1)] + [out_copy(NB - 1, mq, 4) for mq in range(4)])


@jax.jit
def pallas_sequential_preLN__ssm_conv_h3__dense_activation_gelu__prompt_kernel(
    A_q: jax.Array,
    A_k: jax.Array,
    A_v: jax.Array,
    A_shift_k: jax.Array,
    A_ssm_k: jax.Array,
    A_ssm_D: jax.Array,
    B_x: jax.Array,
    B_w1: jax.Array,
    B_b1: jax.Array,
    B_w2: jax.Array,
    B_b2: jax.Array,
):
    del B_x
    any_spec = pl.BlockSpec(memory_space=pl.ANY)
    scratch = [
        pltpu.VMEM((NC, S // 2 + PAD, 128), u32),
        pltpu.VMEM((NC, S // 2 + PAD, 128), u32),
        pltpu.VMEM((NC, S // 2 + PAD, 128), u32),
        pltpu.VMEM((S // 128, D // 2, 128), u32),
        pltpu.VMEM((5, 128, 128), u32),
        pltpu.VMEM((NC, 2, 64, 128), u32),
        [pltpu.VMEM((NB + 1, NR, 128), f32)] * NC,
        [pltpu.VMEM((7, NR + 32, 128), f32)] * NC,
        [pltpu.VMEM((NB, NR + 32, 128), f32)] * NC,
        pltpu.VMEM((NC, NR, 128), f32),
        pltpu.VMEM((NC, 4, 64, 128), u32),
        pltpu.VMEM((NC, B, 128), f32),
        pltpu.VMEM((NC, B // 2, 128), u32),
        pltpu.VMEM((2, NC, B + PAD, 128), f32),
        pltpu.VMEM((NF, B // 2, 128), u32),
        pltpu.VMEM((NC, F // 2, 128), u32),
        pltpu.VMEM((NC, F // 2, 128), u32),
        pltpu.VMEM((S, D), bf16),
        pltpu.VMEM((NC, B, 128), f32),
        pltpu.VMEM((KS, D), bf16),
        pltpu.VMEM((D,), bf16),
        pltpu.VMEM((F,), bf16),
        pltpu.VMEM((D,), bf16),
        pltpu.SemaphoreType.DMA((10,)),
        pltpu.SemaphoreType.REGULAR,
        pltpu.SemaphoreType.DMA((1,)),
    ]
    return pl.pallas_call(
        _kernel,
        in_specs=[any_spec] * 10,
        out_specs=any_spec,
        out_shape=jax.ShapeDtypeStruct((1, S, D), bf16),
        scratch_shapes=scratch,
        compiler_params=pltpu.CompilerParams(
            vmem_limit_bytes=100 * 1024 * 1024,
            disable_bounds_checks=True,
        ),
    )(A_q, A_k, A_v, A_ssm_k, A_shift_k.T, A_ssm_D, B_w1.T, B_b1, B_w2, B_b2)
```

```python
import functools

import numpy as np
import jax
import jax.numpy as jnp
import jax.experimental.pallas as pl
import jax.experimental.pallas.tpu as pltpu

S, D, F = 2048, 512, 1376
KS = 4
B = 256
NB = S // B
N = 2 * B
NC = D // 128
NF = (F + 127) // 128
EPS = 1e-5
f32 = jnp.float32
bf16 = jnp.bfloat16
u32 = jnp.uint32


def _pk2(a, b):
    return pltpu.pack_elementwise([a, b], packed_dtype=bf16)


def _up(x):
    return pltpu.bitcast(x, bf16)


def _half(w, i):
    return pltpu.unpack_elementwise(w, index=i, packed_dtype=bf16, unpacked_dtype=f32)


ZX = NB
ZP = 0


def _ps(t):
    return t - 1


_FINAL = {
    0: [(0, 0)],
    1: [(1, 0), (0, 1)],
    2: [(2, 0), (0, 2), (1, 1), (ZX, 0)],
}
for _t in range(3, NB):
    _FINAL[_t] = [(_t, 0), (0, _t), (1, _t - 1), (_t - 1, 1)]
_FSRC = {0: [], 1: [], 2: [ZP, ZP], 3: [ZP, ZP], 4: [_ps(2), ZP], 5: [_ps(3), ZP],
         6: [_ps(4), _ps(5)], 7: [_ps(6), _ps(7)]}
_EARLY = {
    2: ([(2, 2), (ZX, 0)], _ps(2)),
    3: ([(2, 3), (3, 2)], _ps(3)),
    4: ([(2, 4), (4, 2)], _ps(4)),
    5: ([(3, 3), (ZX, 0)], _ps(5)),
    6: ([(2, 5), (5, 2)], _ps(6)),
    7: ([(3, 4), (4, 3)], _ps(7)),
}
_LOOP = list(range(2, NB))

JS = 144
IO = 72
NR = 576
KOFF = 16
POFF = 8
ZOFF = 24


def _rr(jp, k, n, off=0):
    return pl.ds(JS * jp + k + off, n)


def _ri(jp, k, n, off=0):
    return pl.ds(JS * jp + IO + k + off, n)


def _lut(t, table):
    keys = sorted(table)
    out = jnp.int32(table[keys[-1]])
    for i in keys[-2::-1]:
        out = jnp.where(t == i, jnp.int32(table[i]), out)
    return out


def _ln(x):
    m = jnp.mean(x, axis=-1, keepdims=True)
    xc = x - m
    v = jnp.mean(xc * xc, axis=-1, keepdims=True)
    return xc * jax.lax.rsqrt(v + EPS)


_SINC = [1.0, -1.0 / 6, 1.0 / 120, -1.0 / 5040, 1.0 / 362880, -1.0 / 39916800]
_NT = (((1,), (1,)), ((), ()))
_GC0 = float(np.sqrt(2.0 / np.pi))
_GC1 = _GC0 * 0.044715
RC = 16
PU = 8
PAD = 32

MX = ("b0 k0 Q2 x0 k3 k2 k1 Q1 x1 x3 b1 b2 x2 Q0 b3 b4 b5 i0 b6 Q3 j0 b7 b8 b9 b10 m0 m1 "
      "i2 m2 i1 j2 j1 m3 i3 L0 m4 j3 m5 m6 m7 L1").split()
PR = [x.split() for x in (
    "k0 k1 Q3 Q1 Q0 Q2 k3 k2",
    "x0 x1 i0 x2 x3 j0 i1 j1 i2 j2 i3 j3 L0 L1",
    "b0 b1 b2 b3 b4",
    "b5 x0 x1 x2 k2 k1 k0 x3 k3",
    "Q3 Q2 Q1 Q0 b6 i0 j0 b7 b8 i1 j1 b9 i2 b10 i3 j3 j2",
    "m1 m0 L1 m3 m2 L0",
    "m4 m5 m6 m7",
)]
W1G = [0, 6, 11]
GRP = [(2, 3), (3, 5), (5, 8)]


def _kernel(q_hbm, k_hbm, v_hbm, kk_hbm, sw_hbm, sd_hbm, w1_hbm, b1_hbm, w2_hbm, b2_hbm, o_hbm,
            kw, vw, qw, kkw, c_ref, xb, xf, ps, kp, zprev, ub, qn, hn, hs, gs, w1, w2, ob, kvd,
            sw_ref, sd_ref, b1_ref, b2_ref, sem_in, sem_f, sem_o):

    def kk_copies(t0, t1, sem):
        return [pltpu.make_async_copy(kk_hbm.bitcast(u32).at[:, pl.ds(j * 128, 128)], kkw.at[j], sem)
                for j in range(2 * t0, 2 * t1)]

    def row_copies(src, dst, off, t0, t1, sem):
        n = (t1 - t0) * 128
        return [pltpu.make_async_copy(src.bitcast(u32).at[0, pl.ds(t0 * 128, n), pl.ds(128 * c, 128)],
                                      dst.at[c, pl.ds(off + t0 * 128, n), :], sem) for c in range(NC)]

    def kv_copies(t0, t1, sem):
        return row_copies(k_hbm, kw, 8, t0, t1, sem) + row_copies(v_hbm, vw, 0, t0, t1, sem)

    def q_copies(t0, t1, sem):
        return row_copies(q_hbm, qw, 0, t0, t1, sem)

    def w1_copies(g, sem):
        r0, r1 = 64 * W1G[g], min(64 * W1G[g + 1], F // 2)
        return [pltpu.make_async_copy(w1_hbm.bitcast(u32).at[pl.ds(r0, r1 - r0), pl.ds(128 * c, 128)],
                                      w1.at[c, pl.ds(r0, r1 - r0), :], sem) for c in range(NC)]

    def w2_copies(cp, sem):
        return [pltpu.make_async_copy(w2_hbm.bitcast(u32).at[:, pl.ds(128 * c, 128)], w2.at[c], sem)
                for c in (2 * cp, 2 * cp + 1)]

    def small_copy(i, sem):
        s, d = [(sw_hbm, sw_ref), (sd_hbm, sd_ref), (b1_hbm, b1_ref), (b2_hbm, b2_ref)][i]
        return [pltpu.make_async_copy(s, d, sem)]

    def batch(i):
        sem = sem_in.at[i]
        if i == 0:
            return kk_copies(0, 1, sem) + q_copies(0, 1, sem)
        if i == 1:
            return small_copy(0, sem) + small_copy(1, sem) + kv_copies(0, 1, sem)
        if i == 2:
            return small_copy(2, sem) + small_copy(3, sem) + w1_copies(0, sem)
        if i == 3:
            return kk_copies(1, 2, sem) + kv_copies(1, 2, sem)
        if i == 4:
            return w1_copies(1, sem) + q_copies(1, 2, sem)
        if i in (5, 6):
            return w2_copies(i - 5, sem)
        t0, t1 = GRP[i - 7]
        return kk_copies(t0, t1, sem) + kv_copies(t0, t1, sem) + q_copies(t0, t1, sem)

    def fence():
        pl.semaphore_signal(sem_f, 1)
        pl.semaphore_wait(sem_f, 1)

    def out_copy(t, i=0, n=1):
        rows = pl.ds(t * B + i * (B // n), B // n)
        return pltpu.make_async_copy(ob.at[rows, :], o_hbm.at[0, rows, :], sem_o.at[0])

    def start(cps):
        for cp in cps:
            cp.start()

    def wait(cps):
        for cp in cps:
            cp.wait()

    def gen_consts():
        row = jax.lax.broadcasted_iota(jnp.int32, (32, 128), 0)
        lane = jax.lax.broadcasted_iota(jnp.int32, (32, 128), 1)

        def k0_of(i):
            return jnp.where(i < 32, 2 * i, 2 * i - 63)

        def cosp(p, scale=1.0):
            q = (((p + 512) & 1023) - 512).astype(f32)
            y = (256.0 - jnp.abs(q)) * (np.pi / 512)
            u = y * y
            acc = _SINC[-1] * scale
            for cf in _SINC[-2::-1]:
                acc = acc * u + cf * scale
            return acc * y

        wrap = 128 + ((lane + 127) & 127)
        times = [jnp.where(lane % 2 == 0, lane, wrap), jnp.where(lane % 2 == 1, lane, wrap),
                 2 * lane, 2 * lane + 1]
        for mi in range(4):
            tm = times[mi]
            sg = jnp.where((tm & 2) == 0, 1.0, -1.0)
            re, im = [], []
            for odd in range(2):
                p = (2 * k0_of(2 * row + odd) + 1) * tm
                re.append(cosp(p))
                im.append(cosp(p + 256))
            c_ref[mi, pl.ds(0, 32), :] = _pk2(re[0], re[1])
            c_ref[mi, pl.ds(32, 32), :] = _pk2(im[0], im[1])
            if mi % 2 == 0:
                c_ref[mi, pl.ds(64, 32), :] = _pk2(re[0] * sg, re[1] * sg)
                c_ref[mi, pl.ds(96, 32), :] = _pk2(im[0] * sg, im[1] * sg)
            else:
                c_ref[mi, pl.ds(64, 32), :] = _pk2(im[0] * sg, im[1] * sg)
                c_ref[mi, pl.ds(96, 32), :] = _pk2(re[0] * (-sg), re[1] * (-sg))
        f2 = 2 * k0_of(lane // 2) + 1
        ph = jnp.where(lane % 2 == 1, 256, 0)
        for r in range(4):
            halves = [cosp(f2 * (4 * (2 * row + odd) + r) + ph, 2.0 / N) for odd in range(2)]
            c_ref[4, pl.ds(32 * r, 32), :] = _pk2(halves[0], halves[1])

    def a1_stage(t):
        base = t * 128 if isinstance(t, int) else pl.multiple_of(t * 128, 128)

        def planes(ref, c, off, m0, n):
            w0 = ref[c, pl.ds(off + base + 2 * m0, n, stride=2), :]
            w1_ = ref[c, pl.ds(off + base + 2 * m0 + 1, n, stride=2), :]
            return [_half(w0, 0), _half(w0, 1), _half(w1_, 0), _half(w1_, 1)]

        def ln1(rb, r):
            rows = pl.ds(64 * r + RC * rb, RC)
            cols = [_half(qw[c, pl.ds(base + 2 * RC * rb + r // 2, RC, stride=2), :], r % 2)
                    for c in range(NC)]
            y = _ln(jnp.concatenate(cols, axis=1))
            for c in range(NC):
                qn[c, rows, :] = y[:, 128 * c:128 * (c + 1)]

        def conv(c, rb):
            ls = slice(128 * c, 128 * (c + 1))
            ws = [sw_ref[j:j + 1, ls].astype(f32) for j in range(KS)]
            sd = sd_ref[pl.ds(128 * c, 128)].astype(f32)[None, :]
            m0 = PU * rb
            wm2 = kw[c, pl.ds(8 + base + 2 * m0 - 2, PU, stride=2), :]
            wm1 = kw[c, pl.ds(8 + base + 2 * m0 - 1, PU, stride=2), :]
            kd = [_half(wm2, 1), _half(wm1, 0), _half(wm1, 1)] + planes(kw, c, 8, m0, PU)
            vs = planes(vw, c, 0, m0, PU)
            kvs = []
            for r in range(4):
                ks = None
                for j in range(KS):
                    term = kd[3 + r - j] * ws[j]
                    ks = term if ks is None else ks + term
                kv = ks * vs[r]
                kvs.append(kv)
                kvd[c, pl.ds(64 * r + m0, PU), :] = kv * sd
            for p in range(2):
                xb[c, p, pl.ds(m0, PU), :] = _pk2(kvs[p], kvs[p + 2])

        def xt(c):
            e0 = jnp.dot(_up(c_ref[2]), _up(xb[c, 0]), preferred_element_type=f32)
            e1 = jnp.dot(_up(c_ref[3]), _up(xb[c, 1]), preferred_element_type=f32)
            for h in range(2):
                for part in range(2):
                    a = e0[128 * h + 64 * part:128 * h + 64 * part + 64]
                    b = e1[128 * h + 64 * part:128 * h + 64 * part + 64]
                    rw = _ri if part else _rr
                    xf[c][t, rw(h, 0, 64), :] = a + b
                    xf[c][t, rw(h + 2, 0, 64), :] = a - b

        def kt(c):
            rows = pl.ds(64 * c, 64)
            ka = kkw[2 * t, rows, :]
            kb = pltpu.roll(kkw[2 * t + 1, rows, :], 1, 1)
            ev = (jax.lax.broadcasted_iota(jnp.int32, ka.shape, 1) % 2) == 0
            ke = _up(jnp.where(ev, ka, kb))
            ko = _up(jnp.where(ev, kb, ka))
            e0 = jax.lax.dot_general(_up(c_ref[0]), ke, _NT, preferred_element_type=f32)
            e1 = jax.lax.dot_general(_up(c_ref[1]), ko, _NT, preferred_element_type=f32)
            for h in range(2):
                for part in range(2):
                    a = e0[128 * h + 64 * part:128 * h + 64 * part + 64]
                    b = e1[128 * h + 64 * part:128 * h + 64 * part + 64]
                    rw = _ri if part else _rr
                    kp[c][t, rw(h, 0, 64, KOFF), :] = a + b
                    kp[c][t, rw(h + 2, 0, 64, KOFF), :] = a - b

        units = {}
        mx = {}
        for c in range(NC):
            units["P%d" % c] = [functools.partial(conv, c, rb) for rb in range(64 // PU)]
            mx["x%d" % c] = functools.partial(xt, c)
            mx["k%d" % c] = functools.partial(kt, c)
        for r in range(4):
            units["Q%d" % r] = [functools.partial(ln1, rb, r) for rb in range(64 // RC)]
        need = {"x%d" % c: ["P%d" % c] for c in range(NC)}
        return units, mx, need

    def a2_stage(t):
        sl = t % 2
        first = isinstance(t, int) and t == 0
        if isinstance(t, int):
            base = t * 128
            fin, fs, early = _FINAL[t], _FSRC[t], None
        else:
            base = pl.multiple_of(t * 128, 128)
            fin = [(_lut(t, {s: _FINAL[s][u][0] for s in _LOOP}),
                    _lut(t, {s: _FINAL[s][u][1] for s in _LOOP})) for u in range(4)]
            fs = [_lut(t, {s: _FSRC[s][u] for s in _LOOP}) for u in range(2)]
            early = [(_lut(t, {s: _EARLY[s][0][u][0] for s in _LOOP}),
                      _lut(t, {s: _EARLY[s][0][u][1] for s in _LOOP})) for u in range(2)]
            ed = _lut(t, {s: _EARLY[s][1] for s in _LOOP})

        def cmac(zr, zi, pairs, c, jp, k, n):
            for (i, j) in pairs:
                xr, xi = xf[c][i, _rr(jp, k, n), :], xf[c][i, _ri(jp, k, n), :]
                kr, ki = kp[c][j, _rr(jp, k, n, KOFF), :], kp[c][j, _ri(jp, k, n, KOFF), :]
                pr = xr * kr - xi * ki
                pi = xr * ki + xi * kr
                zr = pr if zr is None else zr + pr
                zi = pi if zi is None else zi + pi
            return zr, zi

        def earlyu(c, jp):
            zr, zi = cmac(None, None, early, c, jp, 0, 64)
            ps[c][ed, _rr(jp, 0, 64, POFF), :] = zr
            ps[c][ed, _ri(jp, 0, 64, POFF), :] = zi

        def final(c, rb):
            zs = []
            for jp in range(4):
                zr = zi = None
                for s in fs:
                    a = ps[c][s, _rr(jp, 8 * rb, 8, POFF), :]
                    b = ps[c][s, _ri(jp, 8 * rb, 8, POFF), :]
                    zr = a if zr is None else zr + a
                    zi = b if zi is None else zi + b
                zr, zi = cmac(zr, zi, fin, c, jp, 8 * rb, 8)
                rs, is_ = _rr(jp, 8 * rb, 8, ZOFF), _ri(jp, 8 * rb, 8, ZOFF)
                if not first:
                    pr, pi = zprev[c, rs, :], zprev[c, is_, :]
                zprev[c, rs, :] = zr
                zprev[c, is_, :] = zi
                if not first:
                    zr, zi = (zr - pi, zi + pr) if rb < 4 else (zr + pi, zi - pr)
                zs.append((zr, zi))
            ar, ai = zs[0][0] + zs[2][0], zs[0][1] + zs[2][1]
            br, bi = zs[0][0] - zs[2][0], zs[0][1] - zs[2][1]
            cr, ci = zs[1][0] + zs[3][0], zs[1][1] + zs[3][1]
            dr, di = zs[1][0] - zs[3][0], zs[1][1] - zs[3][1]
            us = [(ar + cr, ai + ci), (br - di, bi + dr),
                  (ar - cr, ai - ci), (br + di, bi - dr)]
            for r in range(4):
                ub[c, r, pl.ds(8 * rb, 8), :] = _pk2(us[r][0], us[r][1])

        def idft(c, p):
            for r in (p, p + 2):
                y = jnp.dot(_up(c_ref[4, pl.ds(32 * r, 32), :]), _up(ub[c, r]), preferred_element_type=f32)
                rows = pl.ds(64 * r, 64)
                x = _half(qw[c, pl.ds(base + r // 2, 64, stride=2), :], r % 2)
                hs[sl, c, pl.ds(r, 64, stride=4), :] = x + qn[c, rows, :] * (y + kvd[c, rows, :])

        def ln2(p, rb):
            hns = []
            for r in (p, p + 2):
                nat = pl.ds(4 * RC * rb + r, RC, stride=4)
                hns.append(_ln(jnp.concatenate([hs[sl, c, nat, :] for c in range(NC)], axis=1)))
            pk = _pk2(hns[0], hns[1])
            for c in range(NC):
                hn[c, pl.ds(64 * p + RC * rb, RC), :] = pk[:, 128 * c:128 * (c + 1)]

        units = {}
        mx = {}
        for c in range(NC):
            units["E%d" % c] = [functools.partial(earlyu, c, jp) for jp in range(4)] if early else []
            units["F%d" % c] = [functools.partial(final, c, rb) for rb in range(8)]
            mx["i%d" % c] = functools.partial(idft, c, 0)
            mx["j%d" % c] = functools.partial(idft, c, 1)
        for p in range(2):
            units["L%d" % p] = [functools.partial(ln2, p, rb) for rb in range(64 // RC)]
        need = {"i%d" % c: ["E%d" % c, "F%d" % c] for c in range(NC)}
        return units, mx, need

    def b_stage(t):
        sl = t % 2
        obase = t * B if isinstance(t, int) else pl.multiple_of(t * B, B)

        def mm1(n):
            w = min(128, F - 128 * n)
            x = _up(jnp.concatenate([hn[c] for c in range(NC)], axis=1))
            wt = _up(jnp.concatenate([w1[c, pl.ds(64 * n, w // 2), :] for c in range(NC)], axis=1))
            h1 = jax.lax.dot_general(x, wt, _NT, preferred_element_type=f32)
            h1 = h1 + b1_ref[pl.ds(128 * n, w)].astype(f32)[None, :]
            u = h1 * (_GC0 + _GC1 * (h1 * h1))
            g = h1 + h1 * jnp.tanh(u)
            gs[n, :, pl.ds(0, w)] = _pk2(g[:128], g[128:])

        def mm2(i):
            cp, mq = i // 4, i % 4
            rp = pl.ds(32 * mq, 32)
            tiles = [gs[n, rp, :] for n in range(NF - 1)] + [gs[NF - 1, rp, pl.ds(0, F - 128 * (NF - 1))]]
            g = _up(jnp.concatenate(tiles, axis=1))
            o = jnp.concatenate([jnp.dot(g, _up(w2[2 * cp + j]), preferred_element_type=f32)
                                 for j in range(2)], axis=1)
            rs = pl.ds(64 * mq, 64)
            hh = jnp.concatenate([hs[sl, 2 * cp, rs, :], hs[sl, 2 * cp + 1, rs, :]], axis=1)
            bb = b2_ref[pl.ds(256 * cp, 256)].astype(f32)[None, :]
            ob[pl.ds(obase + 64 * mq, 64), pl.ds(256 * cp, 256)] = ((0.5 * o + bb) + hh).astype(bf16)

        mx = {}
        for n in range(NF):
            mx["b%d" % n] = functools.partial(mm1, n)
        for i in range(8):
            mx["m%d" % i] = functools.partial(mm2, i)
        return {}, mx, {}

    def run(order, *stages):
        units, mx, need = {}, {}, {}
        for u, m, n in stages:
            units.update(u)
            mx.update(m)
            need.update(n)
        for o in order:
            if o in units:
                for fn in units[o]:
                    fn()
            else:
                for st in need.get(o, []):
                    for fn in units[st]:
                        fn()
                mx[o]()

    for i in range(7):
        start(batch(i))
        fence()
    for c in range(NC):
        xf[c][ZX] = jnp.zeros(xf[c].shape[1:], f32)
        ps[c][ZP] = jnp.zeros(ps[c].shape[1:], f32)
        kw[c, pl.ds(0, 8), :] = jnp.zeros((8, 128), u32)
    gen_consts()
    wait(batch(0))
    run(PR[0], a1_stage(0))
    start(batch(7))
    wait(batch(1))
    run(PR[1], a1_stage(0), a2_stage(0))
    wait(batch(2))
    run(PR[2], b_stage(0))
    wait(batch(3))
    run(PR[3], a1_stage(1), b_stage(0))
    start(batch(8))
    wait(batch(4))
    run(PR[4], a1_stage(1), a2_stage(1), b_stage(0))
    start(batch(9))
    wait(batch(5))
    run(PR[5], a2_stage(1), b_stage(0))
    wait(batch(6))
    run(PR[6], b_stage(0))
    wait(batch(7))

    def body(it, carry):
        s = _LOOP[0] + it
        out_copy(s - 2).start()
        for gi in (1, 2):
            @pl.when(s == GRP[gi][0])
            def _():
                wait(batch(7 + gi))
        run(MX, b_stage(s - 1), a2_stage(s), a1_stage(s))
        return carry

    jax.lax.fori_loop(0, len(_LOOP), body, 0)

    out_copy(NB - 2).start()
    run(["b%d" % n for n in range(NF)], b_stage(NB - 1))
    for mq in range(4):
        run(["m%d" % mq, "m%d" % (mq + 4)], b_stage(NB - 1))
        out_copy(NB - 1, mq, 4).start()
    wait([out_copy(t) for t in range(NB - 1)] + [out_copy(NB - 1, mq, 4) for mq in range(4)])


@jax.jit
def pallas_sequential_preLN__ssm_conv_h3__dense_activation_gelu__prompt_kernel(
    A_q: jax.Array,
    A_k: jax.Array,
    A_v: jax.Array,
    A_shift_k: jax.Array,
    A_ssm_k: jax.Array,
    A_ssm_D: jax.Array,
    B_x: jax.Array,
    B_w1: jax.Array,
    B_b1: jax.Array,
    B_w2: jax.Array,
    B_b2: jax.Array,
):
    del B_x
    any_spec = pl.BlockSpec(memory_space=pl.ANY)
    scratch = [
        pltpu.VMEM((NC, S // 2 + PAD, 128), u32),
        pltpu.VMEM((NC, S // 2 + PAD, 128), u32),
        pltpu.VMEM((NC, S // 2 + PAD, 128), u32),
        pltpu.VMEM((S // 128, D // 2, 128), u32),
        pltpu.VMEM((5, 128, 128), u32),
        pltpu.VMEM((NC, 2, 64, 128), u32),
        [pltpu.VMEM((NB + 1, NR, 128), f32)] * NC,
        [pltpu.VMEM((7, NR + 32, 128), f32)] * NC,
        [pltpu.VMEM((NB, NR + 32, 128), f32)] * NC,
        pltpu.VMEM((NC, NR + 32, 128), f32),
        pltpu.VMEM((NC, 4, 64, 128), u32),
        pltpu.VMEM((NC, B, 128), f32),
        pltpu.VMEM((NC, B // 2, 128), u32),
        pltpu.VMEM((2, NC, B + PAD, 128), f32),
        pltpu.VMEM((NF, B // 2, 128), u32),
        pltpu.VMEM((NC, F // 2, 128), u32),
        pltpu.VMEM((NC, F // 2, 128), u32),
        pltpu.VMEM((S, D), bf16),
        pltpu.VMEM((NC, B, 128), f32),
        pltpu.VMEM((KS, D), bf16),
        pltpu.VMEM((D,), bf16),
        pltpu.VMEM((F,), bf16),
        pltpu.VMEM((D,), bf16),
        pltpu.SemaphoreType.DMA((10,)),
        pltpu.SemaphoreType.REGULAR,
        pltpu.SemaphoreType.DMA((1,)),
    ]
    return pl.pallas_call(
        _kernel,
        in_specs=[any_spec] * 10,
        out_specs=any_spec,
        out_shape=jax.ShapeDtypeStruct((1, S, D), bf16),
        scratch_shapes=scratch,
        compiler_params=pltpu.CompilerParams(
            vmem_limit_bytes=100 * 1024 * 1024,
            disable_bounds_checks=True,
        ),
    )(A_q, A_k, A_v, A_ssm_k, A_shift_k.T, A_ssm_D, B_w1.T, B_b1, B_w2, B_b2)
```
